```python
import os as _os
_os.environ.setdefault("JAX_PLATFORMS", "cpu")
import jax
import jax.numpy as jnp

def _softmax(x, axis=-1):
    return jax.nn.softmax(x, axis=axis)
def _gelu(x):
    return jax.nn.gelu(x, approximate=True)
def _silu(x):
    return jax.nn.silu(x)
def _sigmoid(x):
    return jax.nn.sigmoid(x)
def _layernorm(x, axis=-1, eps=1e-5):
    m = jnp.mean(x, axis=axis, keepdims=True)
    v = jnp.var(x, axis=axis, keepdims=True)
    return (x - m) / jnp.sqrt(v + eps)
def _scatter_add(tgt, idx, src, axis=0):
    return tgt.at[idx].add(src)
def _segment_sum(src, seg, n):
    return jax.ops.segment_sum(src, seg, n)
class _Rng:
    def __init__(self, key):
        self._k = key
    def _next(self):
        self._k, sub = jax.random.split(self._k)
        return sub
    def normal(self, shape):
        return jax.random.normal(self._next(), shape, dtype=jnp.bfloat16)
    def randint(self, lo, hi, shape):
        return jax.random.randint(self._next(), shape, lo, hi, dtype=jnp.int32)
    def uniform(self, shape, lo=0.0, hi=1.0):
        return jax.random.uniform(self._next(), shape, jnp.bfloat16, lo, hi)
    def permutation(self, n):
        return jax.random.permutation(self._next(), n)


kernel_name = 'sequential_preLN__softmax_full_mha__glu_gated_swiglu__prompt'

def setup_inputs():
    _rng = _Rng(jax.random.key(int.from_bytes(__import__("os").urandom(4), "little")))
    _w = (lambda a: (lambda t: t.astype(jnp.bfloat16) if jnp.issubdtype(t.dtype, jnp.floating) else t)(jnp.asarray(a)))
    def _A_setup():
        B, S, D = 1, 2048, 640
        return {
            "x": _w((lambda *s: _rng.normal(s) * 0.05)(B, S, D)),
            "wqkv": _w((lambda *s: _rng.normal(s) * 0.05)(D, 3 * D)),
            "wo": _w((lambda *s: _rng.normal(s) * 0.05)(D, D)),
        }
    _A_in = _A_setup()

    def _B_setup():
        B, S, D, F = 1, 2048, 640, 1728
        return {
            "x": _w((lambda *s: _rng.normal(s) * 0.05)(B, S, D)),
            "w1": _w((lambda *s: _rng.normal(s) * 0.05)(D, F) * (2.0 / D) ** 0.5),
            "w3": _w((lambda *s: _rng.normal(s) * 0.05)(D, F) * (2.0 / D) ** 0.5),
            "w2": _w((lambda *s: _rng.normal(s) * 0.05)(F, D) * (2.0 / F) ** 0.5),
        }
    _B_in = _B_setup()

    return {
        "A_x": _A_in["x"],
        "A_wqkv": _A_in["wqkv"],
        "A_wo": _A_in["wo"],
        "B_x": _B_in["x"],
        "B_w1": _B_in["w1"],
        "B_w3": _B_in["w3"],
        "B_w2": _B_in["w2"],
    }

def reference(A_x, A_wqkv, A_wo, B_x, B_w1, B_w3, B_w2):
    def _A_ref(x, wqkv, wo):
        B, S, D = x.shape
        H = 32; Dh = D // H
        qkv = (lambda x, *d: x.transpose(*d))((x @ wqkv).reshape(B, S, 3, H, Dh), 2, 0, 3, 1, 4)
        q, k, v = qkv[0], qkv[1], qkv[2]
        scale = Dh ** -0.5
        scores = jnp.einsum("bhqd,bhkd->bhqk", q, k) * scale
        p = _softmax(scores, axis=-1)
        o = jnp.einsum("bhqk,bhkd->bhqd", p, v)
        return (lambda x, *d: x.transpose(*d))(o, 0, 2, 1, 3).reshape(B, S, D) @ wo

    def _B_ref(x, w1, w3, w2):
        gate = jnp.einsum("bsd,df->bsf", x, w1)
        up = jnp.einsum("bsd,df->bsf", x, w3)
        h = _silu(gate) * up
        out = jnp.einsum("bsf,fd->bsd", h, w2)
        return out

    x = A_x
    h = x + _A_ref(_layernorm(x, axis=-1), A_wqkv, A_wo)
    h2 = h + _B_ref(_layernorm(h, axis=-1), B_w1, B_w3, B_w2)
    return h2
```

```python
import functools
import jax
import jax.numpy as jnp
import numpy as np
from jax import lax
import jax.experimental.pallas as pl
import jax.experimental.pallas.tpu as pltpu

S = 2048
D = 640
H = 32
DH = D // H
F = 1728
EPS = 1e-5
QSCALE = float(DH ** -0.5 * np.log2(np.e))
NWIN = 9
VR = 24

RBA = 512
TQ = 512
TK = 128
RBC = 512
NT = S // TQ
NPAIR = H // 2
NPJ = NT * NPAIR
PPI = 2
NFT = F // 128
FREM = F - 128 * NFT

F32 = jnp.float32
BF16 = jnp.bfloat16
NT_DIMS = (((1,), (1,)), ((), ()))


def _layernorm(x):
    mu = jnp.mean(x, axis=-1, keepdims=True)
    xc = x - mu
    var = jnp.mean(xc * xc, axis=-1, keepdims=True)
    return xc * lax.rsqrt(var + EPS)


def _pack(x):
    return pltpu.bitcast(x.astype(BF16), jnp.int32)


def _kernel(x_hbm, wqkv_hbm, wo_hbm, w1_hbm, w3_hbm, w2_hbm, out_hbm,
            x_v, wqkv_v, wo_v, w13_v, w2_v, wqt_v, wvt_v, xn_v,
            qw_v, kw_v, vt_v, s0_v, s1_v, s2_v, s3_v, m_v, ot_v, h_v, hn_v, out_v,
            sem_x, sem_a, sem_w, sem_o):
    nxa = S // RBA

    def x_copy(r):
        return pltpu.make_async_copy(
            x_hbm.at[pl.ds(r * RBA, RBA), :], x_v.at[pl.ds(r * RBA, RBA), :], sem_x.at[r])

    def wqkv_copy(part):
        return pltpu.make_async_copy(
            wqkv_hbm.at[:, pl.ds(part * D, D)], wqkv_v.at[:, pl.ds(part * D, D)], sem_a.at[part])

    wo_copy = pltpu.make_async_copy(wo_hbm, wo_v, sem_w.at[0])
    w2_copy = pltpu.make_async_copy(w2_hbm, w2_v, sem_w.at[1])
    w13_copies = []
    for j in range(NFT):
        w13_copies.append(pltpu.make_async_copy(
            w1_hbm.at[pl.ds(128 * j, 128), :], w13_v.at[pl.ds(256 * j, 128), :], sem_w.at[2]))
        w13_copies.append(pltpu.make_async_copy(
            w3_hbm.at[pl.ds(128 * j, 128), :], w13_v.at[pl.ds(256 * j + 128, 128), :], sem_w.at[2]))
    w13_copies.append(pltpu.make_async_copy(
        w1_hbm.at[pl.ds(128 * NFT, FREM), :], w13_v.at[pl.ds(256 * NFT, FREM), :], sem_w.at[2]))
    w13_copies.append(pltpu.make_async_copy(
        w3_hbm.at[pl.ds(128 * NFT, FREM), :], w13_v.at[pl.ds(256 * NFT + FREM, FREM), :], sem_w.at[2]))
    wqkv_copy(0).start()
    wqkv_copy(2).start()
    x_copy(0).start()
    wqkv_copy(1).start()
    for r in range(1, nxa):
        x_copy(r).start()

    wqkv_copy(0).wait()
    wqt_v[...] = wqkv_v[:, 0:D].T
    wqkv_copy(2).wait()
    wvt_v[...] = wqkv_v[:, 2 * D:3 * D].T
    x_copy(0).wait()
    xn_v[0:RBA, :] = _layernorm(x_v[0:RBA, :].astype(F32)).astype(BF16)
    wqkv_copy(1).wait()

    def phase_a(r, carry):
        rn = jnp.minimum(r + 1, nxa - 1)

        @pl.when(r + 1 < nxa)
        def _():
            x_copy(rn).wait()

        r0 = pl.multiple_of(r * RBA, RBA)
        rn0 = pl.multiple_of(rn * RBA, RBA)
        xn = xn_v[pl.ds(r0, RBA), :]
        xn_next = _layernorm(x_v[pl.ds(rn0, RBA), :].astype(F32)).astype(BF16)
        cols = pl.ds(r0, RBA)
        half = pl.ds(pl.multiple_of(r * (RBA // 2), RBA // 2), RBA // 2)

        k = jnp.dot(xn, wqkv_v[:, D:2 * D], preferred_element_type=F32)
        lane = lax.broadcasted_iota(jnp.int32, (RBA, 128), 1)
        for j in range(5):
            kw_v[j, half, :] = _pack(k[:, 128 * j:128 * (j + 1)])
        for j in range(4):
            kw_v[5 + j, half, :] = _pack(jnp.where(
                lane < 64, k[:, 128 * (j + 1):128 * (j + 2)], k[:, 128 * j:128 * (j + 1)]))

        vt = lax.dot_general(wvt_v[...], xn, NT_DIMS, preferred_element_type=F32)
        row8 = lax.broadcasted_iota(jnp.int32, (8, RBA), 0)
        fill_even = jnp.where(row8 == 4, 1.0, 0.0).astype(F32)
        fill_odd = jnp.where(row8 == 0, 1.0, 0.0).astype(F32)
        for i in range(NPAIR):
            shared = vt[40 * i + 16:40 * i + 24]
            vt_v[2 * i, 0:16, cols] = vt[40 * i:40 * i + 16]
            vt_v[2 * i, 16:24, cols] = jnp.where(row8 < 4, shared, fill_even)
            vt_v[2 * i + 1, 0:8, cols] = jnp.where(row8 >= 4, shared, fill_odd)
            vt_v[2 * i + 1, 8:24, cols] = vt[40 * i + 24:40 * i + 40]

        qt = lax.dot_general(wqt_v[...], xn, NT_DIMS, preferred_element_type=F32) * QSCALE
        qt = _pack(qt)
        for j in range(5):
            qw_v[j, :, cols] = qt[64 * j:64 * (j + 1)]
        for j in range(4):
            qw_v[5 + j, 0:32, cols] = qt[64 * (j + 1):64 * (j + 1) + 32]
            qw_v[5 + j, 32:64, cols] = qt[64 * j + 32:64 * (j + 1)]
        xn_v[pl.ds(rn0, RBA), :] = xn_next
        return carry

    lax.fori_loop(0, nxa, phase_a, 0)
    wo_copy.start()
    for c in w13_copies:
        c.start()
    w2_copy.start()

    def window_of(h):
        f0 = h * DH
        tile = lax.shift_right_logical(f0, 7)
        lo = lax.bitwise_and(f0, 127)
        lane = lax.broadcasted_iota(jnp.int32, (TK // 2, 128), 1)
        mask = lax.bitwise_and(lane - lo, 127) < DH
        return jnp.where(lo + DH > 128, tile + 5, tile), mask

    def q_of(w, t):
        return pltpu.bitcast(qw_v[w, :, pl.ds(pl.multiple_of(t * TQ, TQ), TQ)], BF16)

    def qk_chunk(q, w, mask, c, s_buf, m):
        k = pltpu.bitcast(jnp.where(mask, kw_v[w, c * (TK // 2):(c + 1) * (TK // 2), :], 0), BF16)
        s = jnp.dot(k, q, preferred_element_type=F32)
        s_buf[c * TK:(c + 1) * TK, :] = s
        return jnp.maximum(m, jnp.max(s.reshape(TK // 8, 8, TQ), axis=0))

    def pv_chunk(h, c, s_buf, m, acc):
        s = s_buf[c * TK:(c + 1) * TK, :].reshape(TK // 8, 8, TQ)
        p = jnp.exp2(s - m[None]).reshape(TK, TQ)
        return acc + jnp.dot(vt_v[h, :, c * TK:(c + 1) * TK], p, preferred_element_type=F32)

    def col_max(m):
        return jnp.broadcast_to(jnp.max(m, axis=0, keepdims=True), (8, TQ))

    def pair_out(acc_a, acc_b, i, t):
        oa = acc_a * (1.0 / acc_a[20:21])
        ob = acc_b * (1.0 / acc_b[0:1])
        row8 = lax.broadcasted_iota(jnp.int32, (8, TQ), 0)
        cols = pl.ds(pl.multiple_of(t * TQ, TQ), TQ)
        r0 = pl.multiple_of(i * 40, 8)
        ot_v[pl.ds(r0, 16), cols] = oa[0:16]
        ot_v[pl.ds(r0 + 16, 8), cols] = jnp.where(row8 < 4, oa[16:24], ob[0:8])
        ot_v[pl.ds(r0 + 24, 16), cols] = ob[8:24]

    s_bufs = (s0_v, s1_v, s2_v, s3_v)
    nbuf = 2 * PPI

    def run_jobs(p, do_pv, do_qk):
        for u in range(PPI):
            t = lax.shift_right_logical(p + u, 4)
            i = lax.bitwise_and(p + u, NPAIR - 1)
            t1 = lax.shift_right_logical(p + u + PPI, 4)
            i1 = lax.bitwise_and(p + u + PPI, NPAIR - 1)
            accs = []
            for e in range(2):
                b = 2 * u + e
                h = 2 * i + e
                h1 = 2 * i1 + e
                if do_qk:
                    w, mask = window_of(h1)
                    q = q_of(w, t1)
                    m = jnp.full((8, TQ), -jnp.inf, F32)
                if do_pv:
                    m_cur = m_v[b]
                    acc = jnp.zeros((VR, TQ), F32)
                for c in range(S // TK):
                    if do_pv:
                        acc = pv_chunk(h, c, s_bufs[b], m_cur, acc)
                    if do_qk:
                        m = qk_chunk(q, w, mask, c, s_bufs[b], m)
                if do_qk:
                    m_v[b] = col_max(m)
                if do_pv:
                    accs.append(acc)
            if do_pv:
                pair_out(accs[0], accs[1], i, t)

    assert NPAIR == 16
    run_jobs(jnp.int32(-PPI), False, True)

    nit = NPJ // PPI - 1

    def attn_step(it, carry):
        run_jobs(it * PPI, True, True)
        return carry

    lax.fori_loop(0, nit, attn_step, 0)
    run_jobs(jnp.int32(NPJ - PPI), True, False)

    wo_copy.wait()
    def phase_c1(r2, carry):
        for u in range(2):
            rows = pl.ds(pl.multiple_of((2 * r2 + u) * RBC, RBC), RBC)
            o = ot_v[:, rows].T.astype(BF16)
            h = x_v[rows, :].astype(F32) + jnp.dot(o, wo_v[...], preferred_element_type=F32)
            h_v[rows, :] = h
            hn_v[rows, :] = _layernorm(h).astype(BF16)
        return carry

    lax.fori_loop(0, S // RBC // 2, phase_c1, 0)

    for c in w13_copies:
        c.wait()
    w2_copy.wait()
    nc = S // RBC

    def out_copy(r, slot):
        return pltpu.make_async_copy(
            out_v.at[slot], out_hbm.at[pl.ds(pl.multiple_of(r * RBC, RBC), RBC), :], sem_o.at[slot])

    def phase_c(r, carry):
        r0 = pl.multiple_of(r * RBC, RBC)
        slot = lax.bitwise_and(r, 1)

        @pl.when(r >= 2)
        def _():
            out_copy(r - 2, slot).wait()

        hn = hn_v[pl.ds(r0, RBC), :]
        gu = lax.dot_general(hn, w13_v[...], NT_DIMS, preferred_element_type=F32)
        acts = []
        for j in range(NFT):
            g = gu[:, 256 * j:256 * j + 128]
            u = gu[:, 256 * j + 128:256 * j + 256]
            acts.append((g * jax.nn.sigmoid(g) * u).astype(BF16))
        t = gu[:, 256 * NFT:256 * NFT + 128]
        tail = t * jax.nn.sigmoid(t) * pltpu.roll(t, FREM, 1)
        acts.append(tail[:, 0:FREM].astype(BF16))
        act = jnp.concatenate(acts, axis=1)
        y = h_v[pl.ds(r0, RBC), :] + jnp.dot(act, w2_v[...], preferred_element_type=F32)
        out_v[slot] = y.astype(BF16)
        out_copy(r, slot).start()
        return carry

    lax.fori_loop(0, nc, phase_c, 0)
    for r in range(max(nc - 2, 0), nc):
        out_copy(r, r % 2).wait()


@jax.jit
def pallas_sequential_preLN__softmax_full_mha__glu_gated_swiglu__prompt_kernel(
    A_x: jax.Array,
    A_wqkv: jax.Array,
    A_wo: jax.Array,
    B_x: jax.Array,
    B_w1: jax.Array,
    B_w3: jax.Array,
    B_w2: jax.Array,
):
    del B_x
    x = A_x.reshape(S, D)
    any_spec = pl.BlockSpec(memory_space=pltpu.MemorySpace.HBM)
    out = pl.pallas_call(
        _kernel,
        out_shape=jax.ShapeDtypeStruct((S, D), A_x.dtype),
        in_specs=[any_spec] * 6,
        out_specs=any_spec,
        scratch_shapes=[
            pltpu.VMEM((S, D), BF16),
            pltpu.VMEM((D, 3 * D), BF16),
            pltpu.VMEM((D, D), BF16),
            pltpu.VMEM((2 * F, D), BF16),
            pltpu.VMEM((F, D), BF16),
            pltpu.VMEM((D, D), BF16),
            pltpu.VMEM((D, D), BF16),
            pltpu.VMEM((S, D), BF16),
            pltpu.VMEM((NWIN, 64, S), jnp.int32),
            pltpu.VMEM((NWIN, S // 2, 128), jnp.int32),
            pltpu.VMEM((H, VR, S), F32),
            pltpu.VMEM((S, TQ), F32),
            pltpu.VMEM((S, TQ), F32),
            pltpu.VMEM((S, TQ), F32),
            pltpu.VMEM((S, TQ), F32),
            pltpu.VMEM((2 * PPI, 8, TQ), F32),
            pltpu.VMEM((D, S), F32),
            pltpu.VMEM((S, D), F32),
            pltpu.VMEM((S, D), BF16),
            pltpu.VMEM((2, RBC, D), BF16),
            pltpu.SemaphoreType.DMA((S // RBA,)),
            pltpu.SemaphoreType.DMA((3,)),
            pltpu.SemaphoreType.DMA((3,)),
            pltpu.SemaphoreType.DMA((2,)),
        ],
        compiler_params=pltpu.CompilerParams(vmem_limit_bytes=110 * 1024 * 1024),
    )(x, A_wqkv, A_wo, B_w1.T, B_w3.T, B_w2)
    return out.reshape(A_x.shape)
```

```python
import jax
import jax.numpy as jnp
import numpy as np
from jax import lax
import jax.experimental.pallas as pl
import jax.experimental.pallas.tpu as pltpu

S = 2048
D = 640
H = 32
DH = D // H
F = 1728
EPS = 1e-5
QSCALE = float(DH ** -0.5 * np.log2(np.e))

NWIN = 9
VR = 24
RBA = 512
TQ = 512
TK = 128
RBC = 256
NT = S // TQ
NPAIR = H // 2
NPJ = NT * NPAIR
PPI = 4
PRO_UNROLL = 2
LNS_A = 32
LNS_C = 128
NFT = F // 128
FREM = F - 128 * NFT
FILL_LEAD = 2
FILL_SPILL = 4

F32 = jnp.float32
BF16 = jnp.bfloat16
NT_DIMS = (((1,), (1,)), ((), ()))


def _layernorm(x):
    mu = jnp.mean(x, axis=-1, keepdims=True)
    xc = x - mu
    var = jnp.mean(xc * xc, axis=-1, keepdims=True)
    return xc * lax.rsqrt(var + EPS)


def _pack(x):
    return pltpu.bitcast(x.astype(BF16), jnp.int32)


def _kernel(x_hbm, wqkv_hbm, wo_hbm, w1_hbm, w3_hbm, w2_hbm, out_hbm,
            x_v, wqkv_v, wo_v, w13_v, w2_v, wt_v, xn_v,
            qw_v, kw_v, vt_v, se_v, so_v, m_v, ot_v, h_v, hn_v, out_v,
            sem_x, sem_a, sem_w, sem_o):
    nxa = S // RBA

    def x_copy(r):
        return pltpu.make_async_copy(
            x_hbm.at[pl.ds(r * RBA, RBA), :], x_v.at[pl.ds(r * RBA, RBA), :], sem_x.at[r])

    def wqkv_copy(part):
        return pltpu.make_async_copy(
            wqkv_hbm.at[:, pl.ds(part * D, D)], wqkv_v.at[:, pl.ds(part * D, D)], sem_a.at[part])

    wo_copy = pltpu.make_async_copy(wo_hbm, wo_v, sem_w.at[0])
    w2_copy = pltpu.make_async_copy(w2_hbm, w2_v, sem_w.at[1])
    w13_copies = []
    for j in range(NFT):
        w13_copies.append(pltpu.make_async_copy(
            w1_hbm.at[pl.ds(128 * j, 128), :], w13_v.at[pl.ds(256 * j, 128), :], sem_w.at[2]))
        w13_copies.append(pltpu.make_async_copy(
            w3_hbm.at[pl.ds(128 * j, 128), :], w13_v.at[pl.ds(256 * j + 128, 128), :], sem_w.at[2]))
    w13_copies.append(pltpu.make_async_copy(
        w1_hbm.at[pl.ds(128 * NFT, FREM), :], w13_v.at[pl.ds(256 * NFT, FREM), :], sem_w.at[2]))
    w13_copies.append(pltpu.make_async_copy(
        w3_hbm.at[pl.ds(128 * NFT, FREM), :], w13_v.at[pl.ds(256 * NFT + FREM, FREM), :], sem_w.at[2]))
    x_copy(0).start()
    wqkv_copy(1).start()

    x_copy(0).wait()
    x_copy(1).start()
    xn_v[0:RBA, :] = _layernorm(x_v[0:RBA, :].astype(F32)).astype(BF16)
    wqkv_copy(1).wait()
    x_copy(2).start()
    wqkv_copy(0).start()

    def phase_k(r, carry):
        rn = jnp.minimum(r + 1, nxa - 1)

        @pl.when(r + 1 < nxa)
        def _():
            x_copy(rn).wait()

        @pl.when(r == 1)
        def _():
            x_copy(3).start()
            wqkv_copy(2).start()

        @pl.when(r == 2)
        def _():
            wqkv_copy(0).wait()
            wqkv_copy(2).wait()

        r0 = pl.multiple_of(r * RBA, RBA)
        rn0 = pl.multiple_of(rn * RBA, RBA)
        xn = xn_v[pl.ds(r0, RBA), :]
        src = jnp.where(r == 2, 0, jnp.where(r == 3, 2 * D, D))
        dst = jnp.where(r == 3, 1, 0)
        wt_v[dst] = wqkv_v[:, pl.ds(pl.multiple_of(src, 128), D)].T
        for a in range(RBA // LNS_A):
            rows = pl.ds(pl.multiple_of(rn0 + a * LNS_A, LNS_A), LNS_A)
            xn_v[rows, :] = _layernorm(x_v[rows, :].astype(F32)).astype(BF16)
        half = pl.ds(pl.multiple_of(r * (RBA // 2), RBA // 2), RBA // 2)

        k = jnp.dot(xn, wqkv_v[:, D:2 * D], preferred_element_type=F32)
        lane = lax.broadcasted_iota(jnp.int32, (RBA, 128), 1)
        for j in range(5):
            kw_v[j, half, :] = _pack(k[:, 128 * j:128 * (j + 1)])
        for j in range(4):
            kw_v[5 + j, half, :] = _pack(jnp.where(
                lane < 64, k[:, 128 * (j + 1):128 * (j + 2)], k[:, 128 * j:128 * (j + 1)]))
        return carry

    lax.fori_loop(0, nxa, phase_k, 0)
    def phase_qv(r, carry):
        r0 = pl.multiple_of(r * RBA, RBA)
        xn = xn_v[pl.ds(r0, RBA), :]
        cols = pl.ds(r0, RBA)

        vt = lax.dot_general(wt_v[1], xn, NT_DIMS, preferred_element_type=F32)
        row8 = lax.broadcasted_iota(jnp.int32, (8, RBA), 0)
        fill_even = jnp.where(row8 == 4, 1.0, 0.0).astype(F32)
        fill_odd = jnp.where(row8 == 0, 1.0, 0.0).astype(F32)
        for i in range(NPAIR):
            shared = vt[40 * i + 16:40 * i + 24]
            vt_v[2 * i, 0:16, cols] = vt[40 * i:40 * i + 16]
            vt_v[2 * i, 16:24, cols] = jnp.where(row8 < 4, shared, fill_even)
            vt_v[2 * i + 1, 0:8, cols] = jnp.where(row8 >= 4, shared, fill_odd)
            vt_v[2 * i + 1, 8:24, cols] = vt[40 * i + 24:40 * i + 40]

        qt = lax.dot_general(wt_v[0], xn, NT_DIMS, preferred_element_type=F32) * QSCALE
        qt = _pack(qt)
        for j in range(5):
            qw_v[j, :, cols] = qt[64 * j:64 * (j + 1)]
        for j in range(4):
            qw_v[5 + j, 0:32, cols] = qt[64 * (j + 1):64 * (j + 1) + 32]
            qw_v[5 + j, 32:64, cols] = qt[64 * j + 32:64 * (j + 1)]
        return carry

    lax.fori_loop(0, nxa, phase_qv, 0)
    wo_copy.start()
    for c in w13_copies:
        c.start()
    w2_copy.start()

    def window_of(h):
        f0 = h * DH
        tile = lax.shift_right_logical(f0, 7)
        lo = lax.bitwise_and(f0, 127)
        lane = lax.broadcasted_iota(jnp.int32, (TK // 2, 128), 1)
        mask = lax.bitwise_and(lane - lo, 127) < DH
        return jnp.where(lo + DH > 128, tile + 5, tile), mask

    def q_of(w, t):
        return pltpu.bitcast(qw_v[w, :, pl.ds(pl.multiple_of(t * TQ, TQ), TQ)], BF16)

    def qk_chunk(q, w, mask, c, s_buf, m):
        k = pltpu.bitcast(jnp.where(mask, kw_v[w, c * (TK // 2):(c + 1) * (TK // 2), :], 0), BF16)
        s = jnp.dot(k, q, preferred_element_type=F32)
        s_buf[c * TK:(c + 1) * TK, :] = s
        return jnp.maximum(m, jnp.max(s.reshape(TK // 8, 8, TQ), axis=0))

    def pv_chunk(h, c, s_buf, m, acc):
        s = s_buf[c * TK:(c + 1) * TK, :].reshape(TK // 8, 8, TQ)
        p = jnp.exp2(s - m[None]).reshape(TK, TQ)
        return acc + jnp.dot(vt_v[h, :, c * TK:(c + 1) * TK], p, preferred_element_type=F32)

    def col_max(m):
        return jnp.broadcast_to(jnp.max(m, axis=0, keepdims=True), (8, TQ))

    def pair_out(acc_a, acc_b, i, t):
        oa = acc_a * (1.0 / acc_a[20:21])
        ob = acc_b * (1.0 / acc_b[0:1])
        row8 = lax.broadcasted_iota(jnp.int32, (8, TQ), 0)
        cols = pl.ds(pl.multiple_of(t * TQ, TQ), TQ)
        r0 = pl.multiple_of(i * 40, 8)
        ot_v[pl.ds(r0, 16), cols] = oa[0:16]
        ot_v[pl.ds(r0 + 16, 8), cols] = jnp.where(row8 < 4, oa[16:24], ob[0:8])
        ot_v[pl.ds(r0 + 24, 16), cols] = ob[8:24]

    s_even_odd = (se_v, so_v)

    def pair_jobs(p, u, do_pv, do_qk, side_work=None):
        t = lax.shift_right_logical(p, 4)
        i = lax.bitwise_and(p, NPAIR - 1)
        t1 = lax.shift_right_logical(p + PPI, 4)
        i1 = lax.bitwise_and(p + PPI, NPAIR - 1)
        accs = []
        nchunk = S // TK
        for e in range(2):
            s_buf = s_even_odd[e].at[u]
            b = 2 * u + e
            h = 2 * i + e
            h1 = 2 * i1 + e
            if do_qk:
                w, mask = window_of(h1)
                q = q_of(w, t1)
                m = jnp.full((8, TQ), -jnp.inf, F32)
            if do_pv:
                m_cur = m_v[b]
                acc = jnp.zeros((VR, TQ), F32)
            for c in range(nchunk):
                if do_pv:
                    acc = pv_chunk(h, c, s_buf, m_cur, acc)
                if do_qk:
                    m = qk_chunk(q, w, mask, c, s_buf, m)
                if side_work is not None:
                    side_work(e * nchunk + c)
            if do_qk:
                m_v[b] = col_max(m)
            if do_pv:
                accs.append(acc)
        if do_pv:
            pair_out(accs[0], accs[1], i, t)

    assert NPAIR == 16
    def attn_head(u2, carry):
        for v in range(PRO_UNROLL):
            u = u2 * PRO_UNROLL + v
            pair_jobs(u - PPI, u, False, True)
        return carry

    lax.fori_loop(0, PPI // PRO_UNROLL, attn_head, 0)

    nit = NPJ // PPI - 1

    def attn_step(it, carry):
        for u in range(PPI):
            pair_jobs(it * PPI + u, u, True, True)
        return carry

    lax.fori_loop(0, nit, attn_step, 0)

    wo_copy.wait()
    w2_copy.wait()
    pltpu.make_async_copy(w13_v, w13_v, sem_w.at[2]).wait()

    def o_tile(j, rows):
        return ot_v[128 * j:128 * (j + 1), rows].T.astype(BF16)

    NMAIN = 512
    NKT = D // 128

    def c1_steps(r, js):
        tile_rows = pl.ds(r * TQ, TQ)
        tail = None
        for j in js:
            part = jnp.dot(o_tile(j, tile_rows), wo_v[128 * j:128 * (j + 1), NMAIN:D],
                           preferred_element_type=F32)
            tail = part if tail is None else tail + part
            yield
        for a in range(TQ // 128):
            rows = pl.ds(r * TQ + 128 * a, 128)
            acc = None
            for j in js:
                part = jnp.dot(o_tile(j, rows), wo_v[128 * j:128 * (j + 1), 0:NMAIN],
                               preferred_element_type=F32)
                acc = part if acc is None else acc + part
                if j == js[-1]:
                    acc = jnp.concatenate([acc, tail[128 * a:128 * (a + 1)]], axis=1)
                    base = x_v[rows, :].astype(F32) if js[0] == 0 else h_v[rows, :]
                    h = base + acc
                    h_v[rows, :] = h
                    if r == 0 and 128 * a < RBC:
                        hn_v[rows, :] = _layernorm(h).astype(BF16)
                yield

    first_late = (NPAIR - PPI) * 2 * DH
    early_js = tuple(range(first_late // 128))
    late_js = tuple(range(first_late // 128, NKT))

    def early_work():
        for r in range(NT - 1):
            yield from c1_steps(r, tuple(range(NKT)))
        yield from c1_steps(NT - 1, early_js)

    steps = early_work()
    nsteps = (TQ // 128 + 1) * ((NT - 1) * NKT + len(early_js))
    nchunks = PPI * 2 * (S // TK)
    done = [0]
    for u in range(PPI):
        def side_work(k, u=u):
            target = min(nsteps, (u * 2 * (S // TK) + k + 1 + FILL_LEAD) * nsteps
                         // (nchunks + FILL_SPILL + FILL_LEAD))
            while done[0] < target:
                next(steps)
                done[0] += 1

        pair_jobs(jnp.int32(nit * PPI + u), u, True, False, side_work)
    for _ in steps:
        pass
    for _ in c1_steps(NT - 1, late_js):
        pass

    nc = S // RBC

    def out_copy(r, slot):
        return pltpu.make_async_copy(
            out_v.at[slot], out_hbm.at[pl.ds(pl.multiple_of(r * RBC, RBC), RBC), :], sem_o.at[slot])

    def phase_c(r, carry):
        r0 = pl.multiple_of(r * RBC, RBC)
        slot = lax.bitwise_and(r, 1)

        @pl.when(r >= 2)
        def _():
            out_copy(r - 2, slot).wait()

        hn = hn_v[pl.ds(r0, RBC), :]
        rn0 = pl.multiple_of(jnp.minimum(r + 1, nc - 1) * RBC, RBC)
        for a in range(RBC // LNS_C):
            rows = pl.ds(pl.multiple_of(rn0 + a * LNS_C, LNS_C), LNS_C)
            hn_v[rows, :] = _layernorm(h_v[rows, :]).astype(BF16)
        gu = lax.dot_general(hn, w13_v[...], NT_DIMS, preferred_element_type=F32)
        acts = []
        for j in range(NFT):
            g = gu[:, 256 * j:256 * j + 128]
            u = gu[:, 256 * j + 128:256 * j + 256]
            acts.append((g * jax.nn.sigmoid(g) * u).astype(BF16))
        t = gu[:, 256 * NFT:256 * NFT + 128]
        tail = t * jax.nn.sigmoid(t) * pltpu.roll(t, FREM, 1)
        acts.append(tail[:, 0:FREM].astype(BF16))
        act = jnp.concatenate(acts, axis=1)
        y = h_v[pl.ds(r0, RBC), :] + jnp.dot(act, w2_v[...], preferred_element_type=F32)
        out_v[slot] = y.astype(BF16)
        out_copy(r, slot).start()
        return carry

    lax.fori_loop(0, nc, phase_c, 0)
    for r in range(max(nc - 2, 0), nc):
        out_copy(r, r % 2).wait()


@jax.jit
def pallas_sequential_preLN__softmax_full_mha__glu_gated_swiglu__prompt_kernel(
    A_x: jax.Array,
    A_wqkv: jax.Array,
    A_wo: jax.Array,
    B_x: jax.Array,
    B_w1: jax.Array,
    B_w3: jax.Array,
    B_w2: jax.Array,
):
    del B_x
    x = A_x.reshape(S, D)
    any_spec = pl.BlockSpec(memory_space=pltpu.MemorySpace.HBM)
    out = pl.pallas_call(
        _kernel,
        out_shape=jax.ShapeDtypeStruct((S, D), A_x.dtype),
        in_specs=[any_spec] * 6,
        out_specs=any_spec,
        scratch_shapes=[
            pltpu.VMEM((S, D), BF16),
            pltpu.VMEM((D, 3 * D), BF16),
            pltpu.VMEM((D, D), BF16),
            pltpu.VMEM((2 * F, D), BF16),
            pltpu.VMEM((F, D), BF16),
            pltpu.VMEM((2, D, D), BF16),
            pltpu.VMEM((S, D), BF16),
            pltpu.VMEM((NWIN, 64, S), jnp.int32),
            pltpu.VMEM((NWIN, S // 2, 128), jnp.int32),
            pltpu.VMEM((H, VR, S), F32),
            pltpu.VMEM((PPI, S, TQ), F32),
            pltpu.VMEM((PPI, S, TQ), F32),
            pltpu.VMEM((2 * PPI, 8, TQ), F32),
            pltpu.VMEM((D, S), F32),
            pltpu.VMEM((S, D), F32),
            pltpu.VMEM((S, D), BF16),
            pltpu.VMEM((2, RBC, D), BF16),
            pltpu.SemaphoreType.DMA((S // RBA,)),
            pltpu.SemaphoreType.DMA((3,)),
            pltpu.SemaphoreType.DMA((3,)),
            pltpu.SemaphoreType.DMA((2,)),
        ],
        compiler_params=pltpu.CompilerParams(vmem_limit_bytes=110 * 1024 * 1024),
    )(x, A_wqkv, A_wo, B_w1.T, B_w3.T, B_w2)
    return out.reshape(A_x.shape)
```

```python
import jax
import jax.numpy as jnp
import numpy as np
from jax import lax
import jax.experimental.pallas as pl
import jax.experimental.pallas.tpu as pltpu

S = 2048
D = 640
H = 32
DH = D // H
F = 1728
EPS = 1e-5
QSCALE = float(DH ** -0.5 * np.log2(np.e))

NWIN = 9
VR = 24
RBA = 512
TQ = 512
TK = 128
RBC = 256
NT = S // TQ
NPAIR = H // 2
NPJ = NT * NPAIR
PPI = 4
PRO_UNROLL = 2
LNS_A = 32
LNS_C = 128
NFT = F // 128
FREM = F - 128 * NFT
FILL_LEAD = 2
FILL_SPILL = 2

F32 = jnp.float32
BF16 = jnp.bfloat16
NT_DIMS = (((1,), (1,)), ((), ()))


def _layernorm(x):
    mu = jnp.mean(x, axis=-1, keepdims=True)
    xc = x - mu
    var = jnp.mean(xc * xc, axis=-1, keepdims=True)
    return xc * lax.rsqrt(var + EPS)


def _pack(x):
    return pltpu.bitcast(x.astype(BF16), jnp.int32)


def _kernel(x_hbm, wqkv_hbm, wo_hbm, w1_hbm, w3_hbm, w2_hbm, out_hbm,
            x_v, wqkv_v, wo_v, w13_v, w2_v, wt_v, xn_v,
            qw_v, kw_v, vt_v, se_v, so_v, m_v, ot_v, h_v, hn_v, out_v,
            sem_x, sem_a, sem_w, sem_o):
    nxa = S // RBA

    def x_copy(r):
        return pltpu.make_async_copy(
            x_hbm.at[pl.ds(r * RBA, RBA), :], x_v.at[pl.ds(r * RBA, RBA), :], sem_x.at[r])

    def wqkv_copy(part):
        return pltpu.make_async_copy(
            wqkv_hbm.at[:, pl.ds(part * D, D)], wqkv_v.at[:, pl.ds(part * D, D)], sem_a.at[part])

    wo_copy = pltpu.make_async_copy(wo_hbm, wo_v, sem_w.at[0])
    w2_copy = pltpu.make_async_copy(w2_hbm, w2_v, sem_w.at[1])
    w13_copies = []
    for j in range(NFT):
        w13_copies.append(pltpu.make_async_copy(
            w1_hbm.at[pl.ds(128 * j, 128), :], w13_v.at[pl.ds(256 * j, 128), :], sem_w.at[2]))
        w13_copies.append(pltpu.make_async_copy(
            w3_hbm.at[pl.ds(128 * j, 128), :], w13_v.at[pl.ds(256 * j + 128, 128), :], sem_w.at[2]))
    w13_copies.append(pltpu.make_async_copy(
        w1_hbm.at[pl.ds(128 * NFT, FREM), :], w13_v.at[pl.ds(256 * NFT, FREM), :], sem_w.at[2]))
    w13_copies.append(pltpu.make_async_copy(
        w3_hbm.at[pl.ds(128 * NFT, FREM), :], w13_v.at[pl.ds(256 * NFT + FREM, FREM), :], sem_w.at[2]))
    x_copy(0).start()
    wqkv_copy(1).start()

    x_copy(0).wait()
    x_copy(1).start()
    xn_v[0:RBA, :] = _layernorm(x_v[0:RBA, :].astype(F32)).astype(BF16)
    wqkv_copy(1).wait()
    x_copy(2).start()
    wqkv_copy(0).start()

    def phase_k(r, carry):
        rn = jnp.minimum(r + 1, nxa - 1)

        @pl.when(r + 1 < nxa)
        def _():
            x_copy(rn).wait()

        @pl.when(r == 1)
        def _():
            x_copy(3).start()
            wqkv_copy(2).start()

        @pl.when(r == 2)
        def _():
            wqkv_copy(0).wait()
            wqkv_copy(2).wait()

        r0 = pl.multiple_of(r * RBA, RBA)
        rn0 = pl.multiple_of(rn * RBA, RBA)
        xn = xn_v[pl.ds(r0, RBA), :]
        src = jnp.where(r == 2, 0, jnp.where(r == 3, 2 * D, D))
        dst = jnp.where(r == 3, 1, 0)
        wt_v[dst] = wqkv_v[:, pl.ds(pl.multiple_of(src, 128), D)].T
        for a in range(RBA // LNS_A):
            rows = pl.ds(pl.multiple_of(rn0 + a * LNS_A, LNS_A), LNS_A)
            xn_v[rows, :] = _layernorm(x_v[rows, :].astype(F32)).astype(BF16)
        half = pl.ds(pl.multiple_of(r * (RBA // 2), RBA // 2), RBA // 2)

        k = jnp.dot(xn, wqkv_v[:, D:2 * D], preferred_element_type=F32)
        lane = lax.broadcasted_iota(jnp.int32, (RBA, 128), 1)
        for j in range(5):
            kw_v[j, half, :] = _pack(k[:, 128 * j:128 * (j + 1)])
        for j in range(4):
            kw_v[5 + j, half, :] = _pack(jnp.where(
                lane < 64, k[:, 128 * (j + 1):128 * (j + 2)], k[:, 128 * j:128 * (j + 1)]))
        return carry

    lax.fori_loop(0, nxa, phase_k, 0)

    def phase_qv(r, carry):
        r0 = pl.multiple_of(r * RBA, RBA)
        xn = xn_v[pl.ds(r0, RBA), :]
        cols = pl.ds(r0, RBA)

        vt = lax.dot_general(wt_v[1], xn, NT_DIMS, preferred_element_type=F32)
        row8 = lax.broadcasted_iota(jnp.int32, (8, RBA), 0)
        fill_even = jnp.where(row8 == 4, 1.0, 0.0).astype(F32)
        fill_odd = jnp.where(row8 == 0, 1.0, 0.0).astype(F32)
        for i in range(NPAIR):
            shared = vt[40 * i + 16:40 * i + 24]
            vt_v[2 * i, 0:16, cols] = vt[40 * i:40 * i + 16]
            vt_v[2 * i, 16:24, cols] = jnp.where(row8 < 4, shared, fill_even)
            vt_v[2 * i + 1, 0:8, cols] = jnp.where(row8 >= 4, shared, fill_odd)
            vt_v[2 * i + 1, 8:24, cols] = vt[40 * i + 24:40 * i + 40]

        qt = lax.dot_general(wt_v[0], xn, NT_DIMS, preferred_element_type=F32) * QSCALE
        qt = _pack(qt)
        for j in range(5):
            qw_v[j, :, cols] = qt[64 * j:64 * (j + 1)]
        for j in range(4):
            qw_v[5 + j, 0:32, cols] = qt[64 * (j + 1):64 * (j + 1) + 32]
            qw_v[5 + j, 32:64, cols] = qt[64 * j + 32:64 * (j + 1)]
        return carry

    lax.fori_loop(0, nxa, phase_qv, 0)
    wo_copy.start()
    for c in w13_copies:
        c.start()
    w2_copy.start()

    def window_of(h):
        f0 = h * DH
        tile = lax.shift_right_logical(f0, 7)
        lo = lax.bitwise_and(f0, 127)
        lane = lax.broadcasted_iota(jnp.int32, (TK // 2, 128), 1)
        mask = lax.bitwise_and(lane - lo, 127) < DH
        return jnp.where(lo + DH > 128, tile + 5, tile), mask

    def q_of(w, t):
        return pltpu.bitcast(qw_v[w, :, pl.ds(pl.multiple_of(t * TQ, TQ), TQ)], BF16)

    def qk_chunk(q, w, mask, c, s_buf, m):
        k = pltpu.bitcast(jnp.where(mask, kw_v[w, c * (TK // 2):(c + 1) * (TK // 2), :], 0), BF16)
        s = jnp.dot(k, q, preferred_element_type=F32)
        s_buf[c * TK:(c + 1) * TK, :] = s
        return jnp.maximum(m, jnp.max(s.reshape(TK // 8, 8, TQ), axis=0))

    def pv_chunk(h, c, s_buf, m, acc):
        s = s_buf[c * TK:(c + 1) * TK, :].reshape(TK // 8, 8, TQ)
        p = jnp.exp2(s - m[None]).reshape(TK, TQ)
        return acc + jnp.dot(vt_v[h, :, c * TK:(c + 1) * TK], p, preferred_element_type=F32)

    def col_max(m):
        return jnp.broadcast_to(jnp.max(m, axis=0, keepdims=True), (8, TQ))

    def pair_out(acc_a, acc_b, i, t):
        oa = acc_a * (1.0 / acc_a[20:21])
        ob = acc_b * (1.0 / acc_b[0:1])
        row8 = lax.broadcasted_iota(jnp.int32, (8, TQ), 0)
        cols = pl.ds(pl.multiple_of(t * TQ, TQ), TQ)
        r0 = pl.multiple_of(i * 40, 8)
        ot_v[pl.ds(r0, 16), cols] = oa[0:16]
        ot_v[pl.ds(r0 + 16, 8), cols] = jnp.where(row8 < 4, oa[16:24], ob[0:8])
        ot_v[pl.ds(r0 + 24, 16), cols] = ob[8:24]

    s_even_odd = (se_v, so_v)

    def pair_jobs(p, u, do_pv, do_qk, side_work=None):
        t = lax.shift_right_logical(p, 4)
        i = lax.bitwise_and(p, NPAIR - 1)
        t1 = lax.shift_right_logical(p + PPI, 4)
        i1 = lax.bitwise_and(p + PPI, NPAIR - 1)
        nchunk = S // TK
        bufs = [s_even_odd[e].at[u] for e in range(2)]
        if do_qk:
            wm = [window_of(2 * i1 + e) for e in range(2)]
            qs = [q_of(wm[e][0], t1) for e in range(2)]
            ms = [jnp.full((8, TQ), -jnp.inf, F32) for e in range(2)]
        if do_pv:
            m_cur = [m_v[2 * u + e] for e in range(2)]
            accs = [jnp.zeros((VR, TQ), F32) for e in range(2)]
        if do_pv and do_qk:
            order = [(c, e) for c in range(nchunk) for e in range(2)]
        else:
            order = [(c, e) for e in range(2) for c in range(nchunk)]
        for n, (c, e) in enumerate(order):
            if do_pv:
                accs[e] = pv_chunk(2 * i + e, c, bufs[e], m_cur[e], accs[e])
            if do_qk:
                ms[e] = qk_chunk(qs[e], wm[e][0], wm[e][1], c, bufs[e], ms[e])
                if c == nchunk - 1:
                    m_v[2 * u + e] = col_max(ms[e])
            if side_work is not None:
                side_work(n)
        if do_pv:
            pair_out(accs[0], accs[1], i, t)

    assert NPAIR == 16 and nxa == 4

    def attn_head(u2, carry):
        for v in range(PRO_UNROLL):
            u = u2 * PRO_UNROLL + v
            pair_jobs(u - PPI, u, False, True)
        return carry

    lax.fori_loop(0, PPI // PRO_UNROLL, attn_head, 0)

    nit = NPJ // PPI - 1

    def attn_step(it, carry):
        for u in range(PPI):
            pair_jobs(it * PPI + u, u, True, True)
        return carry

    lax.fori_loop(0, nit, attn_step, 0)

    wo_copy.wait()
    w2_copy.wait()
    pltpu.make_async_copy(w13_v, w13_v, sem_w.at[2]).wait()

    def o_tile(j, rows):
        return ot_v[128 * j:128 * (j + 1), rows].T.astype(BF16)

    NMAIN = 512
    NKT = D // 128

    def c1_steps(r, js):
        tile_rows = pl.ds(r * TQ, TQ)
        tail = None
        for j in js:
            part = jnp.dot(o_tile(j, tile_rows), wo_v[128 * j:128 * (j + 1), NMAIN:D],
                           preferred_element_type=F32)
            tail = part if tail is None else tail + part
            yield
        for a in range(TQ // 128):
            rows = pl.ds(r * TQ + 128 * a, 128)
            acc = None
            for j in js:
                part = jnp.dot(o_tile(j, rows), wo_v[128 * j:128 * (j + 1), 0:NMAIN],
                               preferred_element_type=F32)
                acc = part if acc is None else acc + part
                if j == js[-1]:
                    acc = jnp.concatenate([acc, tail[128 * a:128 * (a + 1)]], axis=1)
                    base = x_v[rows, :].astype(F32) if js[0] == 0 else h_v[rows, :]
                    h = base + acc
                    h_v[rows, :] = h
                    if r == 0 and 128 * a < RBC:
                        hn_v[rows, :] = _layernorm(h).astype(BF16)
                yield

    first_late = (NPAIR - PPI) * 2 * DH
    early_js = tuple(range(first_late // 128))
    late_js = tuple(range(first_late // 128, NKT))

    def early_work():
        for r in range(NT - 1):
            yield from c1_steps(r, tuple(range(NKT)))
        yield from c1_steps(NT - 1, early_js)

    steps = early_work()
    nsteps = (TQ // 128 + 1) * ((NT - 1) * NKT + len(early_js))
    nchunks = PPI * 2 * (S // TK)
    done = [0]
    for u in range(PPI):
        def side_work(k, u=u):
            target = min(nsteps, (u * 2 * (S // TK) + k + 1 + FILL_LEAD) * nsteps
                         // (nchunks + FILL_SPILL + FILL_LEAD))
            while done[0] < target:
                next(steps)
                done[0] += 1

        pair_jobs(jnp.int32(nit * PPI + u), u, True, False, side_work)
    for _ in steps:
        pass
    for _ in c1_steps(NT - 1, late_js):
        pass

    nc = S // RBC

    def out_copy(r, slot):
        return pltpu.make_async_copy(
            out_v.at[slot], out_hbm.at[pl.ds(pl.multiple_of(r * RBC, RBC), RBC), :], sem_o.at[slot])

    def phase_c(r, carry):
        r0 = pl.multiple_of(r * RBC, RBC)
        slot = lax.bitwise_and(r, 1)

        @pl.when(r >= 2)
        def _():
            out_copy(r - 2, slot).wait()

        hn = hn_v[pl.ds(r0, RBC), :]
        rn0 = pl.multiple_of(jnp.minimum(r + 1, nc - 1) * RBC, RBC)
        for a in range(RBC // LNS_C):
            rows = pl.ds(pl.multiple_of(rn0 + a * LNS_C, LNS_C), LNS_C)
            hn_v[rows, :] = _layernorm(h_v[rows, :]).astype(BF16)
        gu = lax.dot_general(hn, w13_v[...], NT_DIMS, preferred_element_type=F32)
        acts = []
        for j in range(NFT):
            g = gu[:, 256 * j:256 * j + 128]
            u = gu[:, 256 * j + 128:256 * j + 256]
            acts.append((g * jax.nn.sigmoid(g) * u).astype(BF16))
        t = gu[:, 256 * NFT:256 * NFT + 128]
        tail = t * jax.nn.sigmoid(t) * pltpu.roll(t, FREM, 1)
        acts.append(tail[:, 0:FREM].astype(BF16))
        act = jnp.concatenate(acts, axis=1)
        y = h_v[pl.ds(r0, RBC), :] + jnp.dot(act, w2_v[...], preferred_element_type=F32)
        out_v[slot] = y.astype(BF16)
        out_copy(r, slot).start()
        return carry

    lax.fori_loop(0, nc, phase_c, 0)
    for r in range(max(nc - 2, 0), nc):
        out_copy(r, r % 2).wait()


@jax.jit
def pallas_sequential_preLN__softmax_full_mha__glu_gated_swiglu__prompt_kernel(
    A_x: jax.Array,
    A_wqkv: jax.Array,
    A_wo: jax.Array,
    B_x: jax.Array,
    B_w1: jax.Array,
    B_w3: jax.Array,
    B_w2: jax.Array,
):
    del B_x
    x = A_x.reshape(S, D)
    hbm_spec = pl.BlockSpec(memory_space=pltpu.MemorySpace.HBM)
    out = pl.pallas_call(
        _kernel,
        out_shape=jax.ShapeDtypeStruct((S, D), A_x.dtype),
        in_specs=[hbm_spec] * 6,
        out_specs=hbm_spec,
        scratch_shapes=[
            pltpu.VMEM((S, D), BF16),
            pltpu.VMEM((D, 3 * D), BF16),
            pltpu.VMEM((D, D), BF16),
            pltpu.VMEM((2 * F, D), BF16),
            pltpu.VMEM((F, D), BF16),
            pltpu.VMEM((2, D, D), BF16),
            pltpu.VMEM((S, D), BF16),
            pltpu.VMEM((NWIN, 64, S), jnp.int32),
            pltpu.VMEM((NWIN, S // 2, 128), jnp.int32),
            pltpu.VMEM((H, VR, S), F32),
            pltpu.VMEM((PPI, S, TQ), F32),
            pltpu.VMEM((PPI, S, TQ), F32),
            pltpu.VMEM((2 * PPI, 8, TQ), F32),
            pltpu.VMEM((D, S), F32),
            pltpu.VMEM((S, D), F32),
            pltpu.VMEM((S, D), BF16),
            pltpu.VMEM((2, RBC, D), BF16),
            pltpu.SemaphoreType.DMA((S // RBA,)),
            pltpu.SemaphoreType.DMA((3,)),
            pltpu.SemaphoreType.DMA((3,)),
            pltpu.SemaphoreType.DMA((2,)),
        ],
        compiler_params=pltpu.CompilerParams(vmem_limit_bytes=110 * 1024 * 1024),
    )(x, A_wqkv, A_wo, B_w1.T, B_w3.T, B_w2)
    return out.reshape(A_x.shape)
```
